```python
import jax
import jax.numpy as jnp

def _softmax(x, axis=-1):
    return jax.nn.softmax(x, axis=axis)
def _gelu(x):
    return jax.nn.gelu(x, approximate=True)
def _silu(x):
    return jax.nn.silu(x)
def _sigmoid(x):
    return jax.nn.sigmoid(x)
def _layernorm(x, axis=-1, eps=1e-5):
    m = jnp.mean(x, axis=axis, keepdims=True)
    v = jnp.var(x, axis=axis, keepdims=True)
    return (x - m) / jnp.sqrt(v + eps)
def _scatter_add(tgt, idx, src, axis=0):
    return tgt.at[idx].add(src)
def _segment_sum(src, seg, n):
    return jax.ops.segment_sum(src, seg, n)
class _Rng:
    def __init__(self, key):
        self._k = key
    def _next(self):
        self._k, sub = jax.random.split(self._k)
        return sub
    def normal(self, shape):
        return jax.random.normal(self._next(), shape, dtype=jnp.bfloat16)
    def randint(self, lo, hi, shape):
        return jax.random.randint(self._next(), shape, lo, hi, dtype=jnp.int32)
    def uniform(self, shape, lo=0.0, hi=1.0):
        return jax.random.uniform(self._next(), shape, jnp.bfloat16, lo, hi)
    def permutation(self, n):
        return jax.random.permutation(self._next(), n)


kernel_name = 'sequential_preLN__grouped_kv_mqa__glu_gated_swiglu__prompt'

def _fwd_setup_inputs():
    _rng = _Rng(jax.random.key(int.from_bytes(__import__("os").urandom(4), "little")))
    _w = (lambda a: (lambda t: t.astype(jnp.bfloat16) if jnp.issubdtype(t.dtype, jnp.floating) else t)(jnp.asarray(a)))
    def _A_setup():
        B, S, D, H = 1, 2048, 512, 32
        Dh = D // H
        return {
            "x": _w((lambda *s: _rng.normal(s) * 0.05)(B, S, D)),
            "wq": _w((lambda *s: _rng.normal(s) * 0.05)(D, H * Dh)),
            "wk": _w((lambda *s: _rng.normal(s) * 0.05)(D, Dh)),
            "wv": _w((lambda *s: _rng.normal(s) * 0.05)(D, Dh)),
            "wo": _w((lambda *s: _rng.normal(s) * 0.05)(H * Dh, D)),
        }
    _A_in = _A_setup()

    def _B_setup():
        B, S, D, F = 1, 2048, 512, 1376
        return {
            "x": _w((lambda *s: _rng.normal(s) * 0.05)(B, S, D)),
            "w1": _w((lambda *s: _rng.normal(s) * 0.05)(D, F) * (2.0 / D) ** 0.5),
            "w3": _w((lambda *s: _rng.normal(s) * 0.05)(D, F) * (2.0 / D) ** 0.5),
            "w2": _w((lambda *s: _rng.normal(s) * 0.05)(F, D) * (2.0 / F) ** 0.5),
        }
    _B_in = _B_setup()

    return {
        "A_x": _A_in["x"],
        "A_wq": _A_in["wq"],
        "A_wk": _A_in["wk"],
        "A_wv": _A_in["wv"],
        "A_wo": _A_in["wo"],
        "B_x": _B_in["x"],
        "B_w1": _B_in["w1"],
        "B_w3": _B_in["w3"],
        "B_w2": _B_in["w2"],
    }

def _fwd_reference(A_x, A_wq, A_wk, A_wv, A_wo, B_x, B_w1, B_w3, B_w2):
    def _A_ref(x, wq, wk, wv, wo):
        B, S, D = x.shape
        H = 32
        Dh = D // H
        q = (lambda x, *d: x.transpose(*d))((x @ wq).reshape(B, S, H, Dh), 0, 2, 1, 3)
        k = x @ wk
        v = x @ wv
        scores = jnp.einsum("bhqd,bkd->bhqk", q, k) * (Dh ** -0.5)
        p = _softmax(scores, axis=-1)
        o = jnp.einsum("bhqk,bkd->bhqd", p, v)
        return (lambda x, *d: x.transpose(*d))(o, 0, 2, 1, 3).reshape(B, S, H * Dh) @ wo

    def _B_ref(x, w1, w3, w2):
        gate = jnp.einsum("bsd,df->bsf", x, w1)
        up = jnp.einsum("bsd,df->bsf", x, w3)
        h = _silu(gate) * up
        out = jnp.einsum("bsf,fd->bsd", h, w2)
        return out

    x = A_x
    h = x + _A_ref(_layernorm(x, axis=-1), A_wq, A_wk, A_wv, A_wo)
    h2 = h + _B_ref(_layernorm(h, axis=-1), B_w1, B_w3, B_w2)
    return h2


def setup_inputs():
    _inp = _fwd_setup_inputs()
    _gk = jax.random.fold_in(jax.random.key(int.from_bytes(__import__("os").urandom(4), "little")), 2**31 - 1)
    _shapes = [[1, 2048, 512]]
    _dtypes = ['bfloat16']
    _gks = jax.random.split(_gk, len(_shapes))
    _gs = [jax.random.normal(k, s, dtype=jnp.dtype(d)) * 0.05 for k, s, d in zip(_gks, _shapes, _dtypes)]
    _inp["grad_out"] = _gs[0]
    return _inp

def reference(A_x, A_wq, A_wk, A_wv, A_wo, B_w1, B_w3, B_w2, B_x, grad_out):
    _const = dict(B_x=B_x)
    def _f(*_d):
        return _fwd_reference(**{'A_x': _d[0], 'A_wq': _d[1], 'A_wk': _d[2], 'A_wv': _d[3], 'A_wo': _d[4], 'B_w1': _d[5], 'B_w3': _d[6], 'B_w2': _d[7], **_const})
    _out, _vjp = jax.vjp(_f, A_x, A_wq, A_wk, A_wv, A_wo, B_w1, B_w3, B_w2)
    _grads = _vjp(grad_out)
    _out0 = jnp.asarray(_out)
    return (_out0, *[jnp.asarray(_g) for _g in _grads])
```

```python
import functools
import jax
import jax.numpy as jnp
from jax import lax
from jax.experimental import pallas as pl
from jax.experimental.pallas import tpu as pltpu

F32 = jnp.float32
BF = jnp.bfloat16
U32 = jnp.uint32

S, D, H, DH, F = 2048, 512, 32, 16, 1376
HD = H * DH
EPS = 1e-5
SCALE = DH ** -0.5

TQ = 128
NT = S // TQ
RT = H * TQ
RC = 512
NC = RT // RC
KBF = 256
NKBF = S // KBF
KBB = 128
NKBB = S // KBB
RB = 16
RC1 = 256
NEG = -1e30

NT_DIMS = (((1,), (1,)), ((), ()))
TN_DIMS = (((0,), (0,)), ((), ()))
TT_DIMS = (((0,), (1,)), ((), ()))


def _dg(a, b, dims):
    return lax.dot_general(a, b, dims, preferred_element_type=F32)


def _nn(a, b):
    return jnp.dot(a, b, preferred_element_type=F32)


def _ln_stats(x):
    mu = jnp.mean(x, axis=-1, keepdims=True)
    xc = x - mu
    var = jnp.mean(xc * xc, axis=-1, keepdims=True)
    rstd = lax.rsqrt(var + EPS)
    return xc * rstd, rstd


def _ln_bwd(dy, xhat, rstd):
    m1 = jnp.mean(dy, axis=-1, keepdims=True)
    m2 = jnp.mean(dy * xhat, axis=-1, keepdims=True)
    return rstd * (dy - m1 - xhat * m2)


def _kernel(x_ref, wq_ref, wk_ref, wv_ref, wo_ref, w1_ref, w3_ref, w2_ref, g_ref,
            h2_ref, dx_ref, dwq_ref, dwk_ref, dwv_ref, dwo_ref, dw1_ref, dw3_ref, dw2_ref,
            xn_scr, wqT_scr, wkvT_scr, k_scr, kT_scr, vaug_scr, vT_scr,
            p_scr, sA, sB, ds0, ds1,
            qcat_scr, doa_scr, qn_scr, don_scr, ol_scr, dqc_scr, oT_scr,
            dqT_scr, dkT_scr, dvT_scr, dh_scr,
            dwo_acc, dw1_acc, dw3_acc, dw2_acc):
    def ln1_body(i, c):
        r = pl.ds(pl.multiple_of(i * RC1, RC1), RC1)
        xhat, _ = _ln_stats(x_ref[r, :].astype(F32))
        xn_scr[r, :] = xhat.astype(BF)
        return c
    lax.fori_loop(0, S // RC1, ln1_body, 0)

    wqT_scr[...] = wq_ref[...].T
    wkvT_scr[0:16, :] = wk_ref[...].T
    wkvT_scr[16:32, :] = wv_ref[...].T

    xn_all = xn_scr[...]
    kv = _dg(xn_all, wkvT_scr[...], NT_DIMS)
    k_scr[...] = kv[:, 0:16].astype(BF)
    lane = lax.broadcasted_iota(jnp.int32, (S, 16), 1)
    ones2 = jnp.where(lane < 2, 1.0, 0.0).astype(F32)
    vaug_scr[...] = jnp.concatenate([kv[:, 16:32], ones2], axis=1).astype(BF)
    kvT = _dg(wkvT_scr[...], xn_all, NT_DIMS)
    kT_scr[...] = kvT[0:16, :].astype(BF)
    vT_scr[0:16, :] = kvT[16:32, :].astype(BF)
    row = lax.broadcasted_iota(jnp.int32, (16, S), 0)
    vT_scr[16:32, :] = jnp.where(row == 0, 1.0, 0.0).astype(BF)

    doa_scr[...] = jnp.zeros_like(doa_scr)
    dkT_scr[...] = jnp.zeros_like(dkT_scr)
    dvT_scr[...] = jnp.zeros_like(dvT_scr)
    dwo_acc[...] = jnp.zeros_like(dwo_acc)
    dw1_acc[...] = jnp.zeros_like(dw1_acc)
    dw3_acc[...] = jnp.zeros_like(dw3_acc)
    dw2_acc[...] = jnp.zeros_like(dw2_acc)

    dsb = [ds0, ds1]

    def tile_body(t, carry):
        rows = pl.ds(pl.multiple_of(t * TQ, TQ), TQ)
        cols = pl.ds(pl.multiple_of(t * TQ, TQ), TQ)
        xn_t = xn_scr[rows, :]

        qT = _dg(wqT_scr[...], xn_t, NT_DIMS) * SCALE
        for h in range(H):
            qcat_scr[:, h * TQ:(h + 1) * TQ] = qT[16 * h:16 * h + 16, :].astype(BF)

        def qt_chunk(c):
            return qcat_scr[:, pl.ds(pl.multiple_of(c * RC, 128), RC)]

        def produce(kb, qt, buf, macc):
            r0 = kb * KBF
            s_new = _nn(k_scr[pl.ds(r0, KBF), :], qt)
            buf[pl.ds(r0, KBF), :] = s_new
            return jnp.maximum(macc, jnp.max(s_new.reshape(KBF // RB, RB, RC), axis=0))

        def consume(kb, c_cur, buf, m, acc):
            r0 = kb * KBF
            p = jnp.exp(buf[pl.ds(r0, KBF), :] - m).astype(BF)
            p_scr[pl.ds(kb * KBF // 2, KBF // 2), pl.ds(pl.multiple_of(c_cur * RC, 128), RC)] = pltpu.bitcast(p, U32)
            return acc + _nn(vT_scr[:, pl.ds(r0, KBF)], p)

        def first(c, buf):
            qt = qt_chunk(c)
            macc = jnp.full((RB, RC), NEG, F32)
            for kb in range(NKBF):
                macc = produce(kb, qt, buf, macc)
            return jnp.max(macc, axis=0, keepdims=True)

        def piped(c_cur, bufC, mC, c_nxt, bufN):
            qt = qt_chunk(c_nxt)
            macc = jnp.full((RB, RC), NEG, F32)
            acc = jnp.zeros((32, RC), F32)
            for kb in range(NKBF):
                macc = produce(kb, qt, bufN, macc)
                acc = consume(kb, c_cur, bufC, mC, acc)
            ol_scr[:, pl.ds(pl.multiple_of(c_cur * RC, 128), RC)] = acc
            return jnp.max(macc, axis=0, keepdims=True)

        def last(c_cur, bufC, mC):
            acc = jnp.zeros((32, RC), F32)
            for kb in range(NKBF):
                acc = consume(kb, c_cur, bufC, mC, acc)
            ol_scr[:, pl.ds(pl.multiple_of(c_cur * RC, 128), RC)] = acc

        mA = first(0, sA)

        def pair_body(c2, mA):
            c = 2 * c2
            mB = piped(c, sA, mA, c + 1, sB)
            return piped(c + 1, sB, mB, c + 2, sA)
        mA = lax.fori_loop(0, NC // 2 - 1, pair_body, mA)
        mB = piped(NC - 2, sA, mA, NC - 1, sB)
        last(NC - 1, sB, mB)

        ol = ol_scr[...]
        inv_l = 1.0 / ol[16:17, :]
        o_cat = ol[0:16, :] * inv_l
        for h in range(H):
            oT_scr[16 * h:16 * h + 16, :] = o_cat[:, h * TQ:(h + 1) * TQ].astype(BF)
        oT = oT_scr[...]

        x_t = x_ref[rows, :].astype(F32)
        h1 = x_t + _dg(oT, wo_ref[...], TN_DIMS)
        hhat, rstd2 = _ln_stats(h1)
        hn = hhat.astype(BF)
        gate = _nn(hn, w1_ref[...])
        up = _nn(hn, w3_ref[...])
        sig = jax.nn.sigmoid(gate)
        silu = gate * sig
        a_bf = (silu * up).astype(BF)
        h2 = h1 + _nn(a_bf, w2_ref[...])
        h2_ref[rows, :] = h2.astype(BF)

        g_t = g_ref[rows, :]
        da = _dg(g_t, w2_ref[...], NT_DIMS)
        dw2_acc[...] += _dg(a_bf, g_t, TN_DIMS)
        dup = (da * silu).astype(BF)
        dgate = (da * up * (sig * (1.0 + gate * (1.0 - sig)))).astype(BF)
        dw1_acc[...] += _dg(hn, dgate, TN_DIMS)
        dw3_acc[...] += _dg(hn, dup, TN_DIMS)
        dhn = _dg(dgate, w1_ref[...], NT_DIMS) + _dg(dup, w3_ref[...], NT_DIMS)
        dh = g_t.astype(F32) + _ln_bwd(dhn, hhat, rstd2)
        dh_scr[rows, :] = dh
        dh_bf = dh.astype(BF)
        dwo_acc[...] += _nn(oT, dh_bf)
        doT = _dg(wo_ref[...], dh_bf, NT_DIMS)

        for h in range(H):
            dqc_scr[:, h * TQ:(h + 1) * TQ] = doT[16 * h:16 * h + 16, :]
        do_cat = dqc_scr[...]
        delta = jnp.sum(do_cat * o_cat, axis=0, keepdims=True)
        d_hi = delta.astype(BF)
        d_lo = (delta - d_hi.astype(F32)).astype(BF)
        doa_scr[0:16, :] = do_cat.astype(BF)
        doa_scr[16:17, :] = -d_hi
        doa_scr[17:18, :] = -d_lo
        don_scr[...] = (do_cat * inv_l).astype(BF)
        qn_scr[...] = (qcat_scr[...].astype(F32) * inv_l).astype(BF)

        def chunk_body(c, cc):
            loc = pl.multiple_of(c * RC, 128)
            doa = doa_scr[:, pl.ds(loc, RC)]
            qn = qn_scr[:, pl.ds(loc, RC)]
            don = don_scr[:, pl.ds(loc, RC)]

            def loadp(kb):
                return pltpu.bitcast(p_scr[pl.ds(kb * KBB // 2, KBB // 2), pl.ds(loc, RC)], BF)

            def stageA(kb):
                r0 = kb * KBB
                gm = _nn(vaug_scr[pl.ds(r0, KBB), :], doa)
                dsb[kb % 2][...] = pltpu.bitcast((loadp(kb).astype(F32) * gm).astype(BF), U32)

            def stageB(kb, dq_acc):
                r0 = kb * KBB
                ds = pltpu.bitcast(dsb[kb % 2][...], BF)
                p = loadp(kb)
                dq_acc = dq_acc + _nn(kT_scr[:, pl.ds(r0, KBB)], ds)
                dkT_scr[:, pl.ds(r0, KBB)] += _dg(qn, ds, NT_DIMS)
                dvT_scr[:, pl.ds(r0, KBB)] += _dg(don, p, NT_DIMS)
                return dq_acc

            dq_acc = jnp.zeros((16, RC), F32)
            stageA(0)
            for kb in range(NKBB):
                if kb + 1 < NKBB:
                    stageA(kb + 1)
                dq_acc = stageB(kb, dq_acc)
            dqc_scr[:, pl.ds(loc, RC)] = dq_acc
            return cc
        lax.fori_loop(0, NC, chunk_body, 0)

        dq_cat = dqc_scr[...] * (inv_l * SCALE)
        for h in range(H):
            dqT_scr[16 * h:16 * h + 16, cols] = dq_cat[:, h * TQ:(h + 1) * TQ].astype(BF)
        return carry

    lax.fori_loop(0, NT, tile_body, 0)

    xn_all = xn_scr[...]
    dqT_all = dqT_scr[...]
    dkvT = jnp.concatenate([dkT_scr[...], dvT_scr[...]], axis=0).astype(BF)
    dwq_ref[...] = _dg(xn_all, dqT_all, TT_DIMS).astype(BF)
    dwkv = _dg(xn_all, dkvT, TT_DIMS)
    dwk_ref[...] = dwkv[:, 0:16].astype(BF)
    dwv_ref[...] = dwkv[:, 16:32].astype(BF)
    dwo_ref[...] = dwo_acc[...].astype(BF)
    dw1_ref[...] = dw1_acc[...].astype(BF)
    dw3_ref[...] = dw3_acc[...].astype(BF)
    dw2_ref[...] = dw2_acc[...].astype(BF)
    doa_scr[:, 0:S] = jnp.concatenate([dkvT], axis=0)

    def ep_body(i, c):
        off = pl.multiple_of(i * RC1, RC1)
        r = pl.ds(off, RC1)
        dxn = _dg(dqT_scr[:, pl.ds(off, RC1)], wqT_scr[...], TN_DIMS) + \
              _dg(doa_scr[:, pl.ds(off, RC1)], wkvT_scr[...], TN_DIMS)
        xhat, rstd1 = _ln_stats(x_ref[r, :].astype(F32))
        dx = dh_scr[r, :] + _ln_bwd(dxn, xhat, rstd1)
        dx_ref[r, :] = dx.astype(BF)
        return c
    lax.fori_loop(0, S // RC1, ep_body, 0)


def _scratch():
    return [
        pltpu.VMEM((S, D), BF),
        pltpu.VMEM((HD, D), BF),
        pltpu.VMEM((32, D), BF),
        pltpu.VMEM((S, 16), BF),
        pltpu.VMEM((16, S), BF),
        pltpu.VMEM((S, 32), BF),
        pltpu.VMEM((32, S), BF),
        pltpu.VMEM((S // 2, RT), U32),
        pltpu.VMEM((S, RC), F32),
        pltpu.VMEM((S, RC), F32),
        pltpu.VMEM((KBB // 2, RC), U32),
        pltpu.VMEM((KBB // 2, RC), U32),
        pltpu.VMEM((16, RT), BF),
        pltpu.VMEM((32, RT), BF),
        pltpu.VMEM((16, RT), BF),
        pltpu.VMEM((16, RT), BF),
        pltpu.VMEM((32, RT), F32),
        pltpu.VMEM((16, RT), F32),
        pltpu.VMEM((HD, TQ), BF),
        pltpu.VMEM((HD, S), BF),
        pltpu.VMEM((16, S), F32),
        pltpu.VMEM((16, S), F32),
        pltpu.VMEM((S, D), F32),
        pltpu.VMEM((HD, D), F32),
        pltpu.VMEM((D, F), F32),
        pltpu.VMEM((D, F), F32),
        pltpu.VMEM((F, D), F32),
    ]


@jax.jit
def pallas_sequential_preLN__grouped_kv_mqa__glu_gated_swiglu__prompt_kernel(
    A_x, A_wq, A_wk, A_wv, A_wo, B_x, B_w1, B_w3, B_w2, grad_out):
    x = A_x.reshape(S, D)
    g = grad_out.reshape(S, D)
    out_shape = (
        jax.ShapeDtypeStruct((S, D), BF), jax.ShapeDtypeStruct((S, D), BF),
        jax.ShapeDtypeStruct((D, HD), BF), jax.ShapeDtypeStruct((D, DH), BF), jax.ShapeDtypeStruct((D, DH), BF),
        jax.ShapeDtypeStruct((HD, D), BF), jax.ShapeDtypeStruct((D, F), BF), jax.ShapeDtypeStruct((D, F), BF),
        jax.ShapeDtypeStruct((F, D), BF),
    )
    outs = pl.pallas_call(
        _kernel, out_shape=out_shape, scratch_shapes=_scratch(),
        compiler_params=pltpu.CompilerParams(vmem_limit_bytes=120 * 1024 * 1024),
    )(x, A_wq, A_wk, A_wv, A_wo, B_w1, B_w3, B_w2, g)
    h2, dx = outs[0].reshape(1, S, D), outs[1].reshape(1, S, D)
    return (h2, dx) + tuple(outs[2:])
```

```python
import contextlib
import functools
import jax
import jax.numpy as jnp
from jax import lax
from jax.experimental import pallas as pl
from jax.experimental.pallas import tpu as pltpu

F32 = jnp.float32
BF = jnp.bfloat16
U32 = jnp.uint32

S, D, H, DH, F = 2048, 512, 32, 16, 1376
HD = H * DH
EPS = 1e-5
SCALE = DH ** -0.5
NEG = -1e30

NT_DIMS = (((1,), (1,)), ((), ()))
TN_DIMS = (((0,), (0,)), ((), ()))
TT_DIMS = (((0,), (1,)), ((), ()))

DEFAULT_CFG = dict(
    TQ=256,
    RC=512,
    KBF=128,
    KBB=128,
    RB=16,
    RC1=256,
    BWD_ORDER='dv,dk,dq',
    FWD_ORDER='pc',
    BWD_DIST=2,
    BWD_APOS=0,
    PROFILE=False,
)


def _dg(a, b, dims):
    return lax.dot_general(a, b, dims, preferred_element_type=F32)


def _nn(a, b):
    return jnp.dot(a, b, preferred_element_type=F32)


def _ln_stats(x):
    mu = jnp.mean(x, axis=-1, keepdims=True)
    xc = x - mu
    var = jnp.mean(xc * xc, axis=-1, keepdims=True)
    rstd = lax.rsqrt(var + EPS)
    return xc * rstd, rstd


def _ln_bwd(dy, xhat, rstd):
    m1 = jnp.mean(dy, axis=-1, keepdims=True)
    m2 = jnp.mean(dy * xhat, axis=-1, keepdims=True)
    return rstd * (dy - m1 - xhat * m2)


def _make_kernel(cfg):
    TQ, RC, KBF, KBB, RB, RC1 = cfg['TQ'], cfg['RC'], cfg['KBF'], cfg['KBB'], cfg['RB'], cfg['RC1']
    NT = S // TQ
    RT = H * TQ
    NC = RT // RC
    NKBF = S // KBF
    NKBB = S // KBB
    BWD_ORDER = cfg['BWD_ORDER'].split(',')
    BWD_DIST = cfg['BWD_DIST']
    BWD_APOS = cfg['BWD_APOS']
    NDS = min(n for n in range(BWD_DIST + 1, NKBB + 1) if NKBB % n == 0)

    def scope(name):
        return jax.named_scope(name) if cfg['PROFILE'] else contextlib.nullcontext()

    def kernel(x_hbm, wq_hbm, wkt_hbm, wvt_hbm, wo_hbm, w1t_hbm, w3t_hbm, w2_hbm, g_hbm,
               h2_hbm, dx_hbm, dwq_hbm, dwkt_hbm, dwvt_hbm, dwo_hbm, dw1t_hbm, dw3t_hbm, dw2_hbm,
               x_ref, wq_ref, wkt_ref, wvt_ref, wo_ref, w1t_ref, w3t_ref, w2_ref, g_ref,
               h2_ref, dx_ref, dwq_ref, dwkt_ref, dwvt_ref, dwo_ref, dw1t_ref, dw3t_ref, dw2_ref,
               in_sems, out_sems,
               xn_scr, wqT_scr, wkvT_scr, k_scr, kT_scr, vaug_scr, vT_scr,
               p_scr, sA, sB,
               qcat_scr, doa_scr, qn_scr, don_scr, ol_scr, dqc_scr, oT_scr,
               dqT_scr, dkT_scr, dvT_scr, dh_scr,
               dwo_acc, dw1t_acc, dw3t_acc, dw2_acc, *dsb):
        in_pairs = [(x_hbm, x_ref), (wq_hbm, wq_ref), (wkt_hbm, wkt_ref), (wvt_hbm, wvt_ref), (wo_hbm, wo_ref),
                    (w1t_hbm, w1t_ref), (w3t_hbm, w3t_ref), (w2_hbm, w2_ref), (g_hbm, g_ref)]
        in_copies = [pltpu.make_async_copy(src, dst, in_sems.at[i]) for i, (src, dst) in enumerate(in_pairs)]
        for cp in in_copies:
            cp.start()

        with scope('prologue'):
            for cp in in_copies[0:4]:
                cp.wait()
            def ln1_body(i, c):
                r = pl.ds(pl.multiple_of(i * RC1, RC1), RC1)
                xhat, _ = _ln_stats(x_ref[r, :].astype(F32))
                xn_scr[r, :] = xhat.astype(BF)
                return c
            lax.fori_loop(0, S // RC1, ln1_body, 0)

            wqT_scr[...] = wq_ref[...].T
            wkvT_scr[0:16, :] = wkt_ref[...]
            wkvT_scr[16:32, :] = wvt_ref[...]

            xn_all = xn_scr[...]
            kv = _dg(xn_all, wkvT_scr[...], NT_DIMS)
            k_scr[...] = kv[:, 0:16].astype(BF)
            lane = lax.broadcasted_iota(jnp.int32, (S, 16), 1)
            ones2 = jnp.where(lane < 2, 1.0, 0.0).astype(F32)
            vaug_scr[...] = jnp.concatenate([kv[:, 16:32], ones2], axis=1).astype(BF)
            kvT = _dg(wkvT_scr[...], xn_all, NT_DIMS)
            kT_scr[...] = kvT[0:16, :].astype(BF)
            vT_scr[0:16, :] = kvT[16:32, :].astype(BF)
            row = lax.broadcasted_iota(jnp.int32, (16, S), 0)
            vT_scr[16:32, :] = jnp.where(row == 0, 1.0, 0.0).astype(BF)

            doa_scr[...] = jnp.zeros_like(doa_scr)
            dkT_scr[...] = jnp.zeros_like(dkT_scr)
            dvT_scr[...] = jnp.zeros_like(dvT_scr)
            dwo_acc[...] = jnp.zeros_like(dwo_acc)
            dw1t_acc[...] = jnp.zeros_like(dw1t_acc)
            dw3t_acc[...] = jnp.zeros_like(dw3t_acc)
            dw2_acc[...] = jnp.zeros_like(dw2_acc)

        def compute_qcat(t, slot):
            xn_t = xn_scr[pl.ds(pl.multiple_of(t * TQ, TQ), TQ), :]
            qT = _dg(wqT_scr[...], xn_t, NT_DIMS) * SCALE
            for h in range(H):
                qcat_scr[slot, :, h * TQ:(h + 1) * TQ] = qT[16 * h:16 * h + 16, :].astype(BF)

        def qt_chunk(slot, c):
            return qcat_scr[slot, :, pl.ds(pl.multiple_of(c * RC, 128), RC)]

        def produce(kb, qt, buf, macc):
            r0 = kb * KBF
            s_new = _nn(k_scr[pl.ds(r0, KBF), :], qt)
            buf[pl.ds(r0, KBF), :] = s_new
            return jnp.maximum(macc, jnp.max(s_new.reshape(KBF // RB, RB, RC), axis=0))

        def consume(kb, c_cur, buf, m, acc):
            r0 = kb * KBF
            p = jnp.exp(buf[pl.ds(r0, KBF), :] - m).astype(BF)
            p_scr[pl.ds(kb * KBF // 2, KBF // 2),
                  pl.ds(pl.multiple_of(c_cur * RC, 128), RC)] = pltpu.bitcast(p, U32)
            return acc + _nn(vT_scr[:, pl.ds(r0, KBF)], p)

        def first(qt, buf):
            macc = jnp.full((RB, RC), NEG, F32)
            for kb in range(NKBF):
                macc = produce(kb, qt, buf, macc)
            return jnp.max(macc, axis=0, keepdims=True)

        def piped(c_cur, bufC, mC, qt_nxt, bufN):
            macc = jnp.full((RB, RC), NEG, F32)
            acc = jnp.zeros((32, RC), F32)
            for kb in range(NKBF):
                macc = produce(kb, qt_nxt, bufN, macc)
                acc = consume(kb, c_cur, bufC, mC, acc)
            ol_scr[:, pl.ds(pl.multiple_of(c_cur * RC, 128), RC)] = acc
            return jnp.max(macc, axis=0, keepdims=True)

        compute_qcat(0, 0)
        m_init = first(qt_chunk(0, 0), sA)
        for cp in in_copies[4:]:
            cp.wait()

        def h2_copy(t):
            r = pl.ds(pl.multiple_of(t * TQ, TQ), TQ)
            return pltpu.make_async_copy(h2_ref.at[r, :], h2_hbm.at[r, :], out_sems.at[0])

        def tile_body(t, mA):
            rows = pl.ds(pl.multiple_of(t * TQ, TQ), TQ)
            cols = pl.ds(pl.multiple_of(t * TQ, TQ), TQ)
            slot = lax.rem(t, 2)
            nslot = 1 - slot

            with scope('qT'):
                compute_qcat(jnp.minimum(t + 1, NT - 1), nslot)

            with scope('attn_fwd'):
                def pair_body(c2, mA):
                    c = 2 * c2
                    mB = piped(c, sA, mA, qt_chunk(slot, c + 1), sB)
                    return piped(c + 1, sB, mB, qt_chunk(slot, c + 2), sA)
                mA = lax.fori_loop(0, NC // 2 - 1, pair_body, mA)
                mB = piped(NC - 2, sA, mA, qt_chunk(slot, NC - 1), sB)
                mA_next = piped(NC - 1, sB, mB, qt_chunk(nslot, 0), sA)

            with scope('norm'):
                ol = ol_scr[...]
                inv_l = 1.0 / ol[16:17, :]
                o_cat = ol[0:16, :] * inv_l
                for h in range(H):
                    oT_scr[16 * h:16 * h + 16, :] = o_cat[:, h * TQ:(h + 1) * TQ].astype(BF)
                oT = oT_scr[...]

            with scope('dense_fwd'):
                x_t = x_ref[rows, :].astype(F32)
                h1 = x_t + _dg(oT, wo_ref[...], TN_DIMS)
                hhat, rstd2 = _ln_stats(h1)
                hn = hhat.astype(BF)
                gate = _dg(hn, w1t_ref[...], NT_DIMS)
                up = _dg(hn, w3t_ref[...], NT_DIMS)
                sig = jax.nn.sigmoid(gate)
                silu = gate * sig
                a_bf = (silu * up).astype(BF)
                h2 = h1 + _nn(a_bf, w2_ref[...])
                h2_ref[rows, :] = h2.astype(BF)
                h2_copy(t).start()

            with scope('dense_bwd'):
                g_t = g_ref[rows, :]
                da = _dg(g_t, w2_ref[...], NT_DIMS)
                dw2_acc[...] += _dg(a_bf, g_t, TN_DIMS)
                dup = (da * silu).astype(BF)
                dgate = (da * up * (sig * (1.0 + gate * (1.0 - sig)))).astype(BF)
                dw1t_acc[...] += _dg(dgate, hn, TN_DIMS)
                dw3t_acc[...] += _dg(dup, hn, TN_DIMS)
                dhn = _nn(dgate, w1t_ref[...]) + _nn(dup, w3t_ref[...])
                dh = g_t.astype(F32) + _ln_bwd(dhn, hhat, rstd2)
                dh_scr[rows, :] = dh
                dh_bf = dh.astype(BF)
                dwo_acc[...] += _nn(oT, dh_bf)
                doT = _dg(wo_ref[...], dh_bf, NT_DIMS)

            with scope('scatter'):
                for h in range(H):
                    dqc_scr[:, h * TQ:(h + 1) * TQ] = doT[16 * h:16 * h + 16, :]
                do_cat = dqc_scr[...]
                delta = jnp.sum(do_cat * o_cat, axis=0, keepdims=True)
                d_hi = delta.astype(BF)
                d_lo = (delta - d_hi.astype(F32)).astype(BF)
                doa_scr[0:16, :] = do_cat.astype(BF)
                doa_scr[16:17, :] = -d_hi
                doa_scr[17:18, :] = -d_lo
                don_scr[...] = (do_cat * inv_l).astype(BF)
                qn_scr[...] = (qcat_scr[slot].astype(F32) * inv_l).astype(BF)

            with scope('attn_bwd'):
                def loadp(kb, loc):
                    return pltpu.bitcast(p_scr[pl.ds(kb * KBB // 2, KBB // 2), pl.ds(loc, RC)], BF)

                def stageA(kb, loc):
                    r0 = kb * KBB
                    gm = _nn(vaug_scr[pl.ds(r0, KBB), :], doa_scr[:, pl.ds(loc, RC)])
                    dsb[kb % NDS][...] = pltpu.bitcast((loadp(kb, loc).astype(F32) * gm).astype(BF), U32)

                def chunk_body(c, cc):
                    loc = pl.multiple_of(c * RC, 128)
                    loc_nxt = pl.multiple_of(jnp.minimum(c + 1, NC - 1) * RC, 128)
                    qn = qn_scr[:, pl.ds(loc, RC)]
                    don = don_scr[:, pl.ds(loc, RC)]

                    def stageB(kb, dq_acc):
                        r0 = kb * KBB
                        for pos, what in enumerate(BWD_ORDER + ['end']):
                            if pos == BWD_APOS:
                                if kb + BWD_DIST < NKBB:
                                    stageA(kb + BWD_DIST, loc)
                                else:
                                    stageA(kb + BWD_DIST - NKBB, loc_nxt)
                            if what == 'end':
                                continue
                            if what == 'dq':
                                ds = pltpu.bitcast(dsb[kb % NDS][...], BF)
                                dq_acc = dq_acc + _nn(kT_scr[:, pl.ds(r0, KBB)], ds)
                            elif what == 'dk':
                                ds = pltpu.bitcast(dsb[kb % NDS][...], BF)
                                dkT_scr[:, pl.ds(r0, KBB)] += _dg(qn, ds, NT_DIMS)
                            else:
                                dvT_scr[:, pl.ds(r0, KBB)] += _dg(don, loadp(kb, loc), NT_DIMS)
                        return dq_acc

                    dq_acc = jnp.zeros((16, RC), F32)
                    for kb in range(NKBB):
                        dq_acc = stageB(kb, dq_acc)
                    dqc_scr[:, pl.ds(loc, RC)] = dq_acc
                    return cc
                for kb in range(BWD_DIST):
                    stageA(kb, 0)
                lax.fori_loop(0, NC, chunk_body, 0)

            dq_cat = dqc_scr[...] * (inv_l * SCALE)
            for h in range(H):
                dqT_scr[16 * h:16 * h + 16, cols] = dq_cat[:, h * TQ:(h + 1) * TQ].astype(BF)
            return mA_next

        lax.fori_loop(0, NT, tile_body, m_init)

        with scope('epilogue'):
            dwo_ref[...] = dwo_acc[...].astype(BF)
            dw1t_ref[...] = dw1t_acc[...].astype(BF)
            dw3t_ref[...] = dw3t_acc[...].astype(BF)
            dw2_ref[...] = dw2_acc[...].astype(BF)
            w_copies = [pltpu.make_async_copy(dwo_ref, dwo_hbm, out_sems.at[2]),
                        pltpu.make_async_copy(dw1t_ref, dw1t_hbm, out_sems.at[3]),
                        pltpu.make_async_copy(dw3t_ref, dw3t_hbm, out_sems.at[4]),
                        pltpu.make_async_copy(dw2_ref, dw2_hbm, out_sems.at[5])]
            for cp in w_copies:
                cp.start()

            xn_all = xn_scr[...]
            dqT_all = dqT_scr[...]
            doa_scr[0:16, 0:S] = dkT_scr[...].astype(BF)
            doa_scr[16:32, 0:S] = dvT_scr[...].astype(BF)
            dkvT = doa_scr[:, 0:S]
            dwq_ref[...] = _dg(xn_all, dqT_all, TT_DIMS).astype(BF)
            dwkvt = _nn(dkvT, xn_all)
            dwkt_ref[...] = dwkvt[0:16, :].astype(BF)
            dwvt_ref[...] = dwkvt[16:32, :].astype(BF)
            w_copies += [pltpu.make_async_copy(dwq_ref, dwq_hbm, out_sems.at[6]),
                         pltpu.make_async_copy(dwkt_ref, dwkt_hbm, out_sems.at[7]),
                         pltpu.make_async_copy(dwvt_ref, dwvt_hbm, out_sems.at[8])]
            for cp in w_copies[4:]:
                cp.start()

            def dx_copy(i):
                r = pl.ds(pl.multiple_of(i * RC1, RC1), RC1)
                return pltpu.make_async_copy(dx_ref.at[r, :], dx_hbm.at[r, :], out_sems.at[1])

            def ep_body(i, c):
                off = pl.multiple_of(i * RC1, RC1)
                r = pl.ds(off, RC1)
                dxn = (_dg(dqT_scr[:, pl.ds(off, RC1)], wqT_scr[...], TN_DIMS) +
                       _dg(doa_scr[:, pl.ds(off, RC1)], wkvT_scr[...], TN_DIMS))
                xhat, rstd1 = _ln_stats(x_ref[r, :].astype(F32))
                dx = dh_scr[r, :] + _ln_bwd(dxn, xhat, rstd1)
                dx_ref[r, :] = dx.astype(BF)
                dx_copy(i).start()
                return c
            lax.fori_loop(0, S // RC1, ep_body, 0)

            def wait_h2(t, c):
                h2_copy(t).wait()
                return c
            lax.fori_loop(0, NT, wait_h2, 0)

            def wait_dx(i, c):
                dx_copy(i).wait()
                return c
            lax.fori_loop(0, S // RC1, wait_dx, 0)
            for cp in w_copies:
                cp.wait()

    in_shapes = [(S, D), (D, HD), (DH, D), (DH, D), (HD, D), (F, D), (F, D), (F, D), (S, D)]
    out_shapes = [(S, D), (S, D), (D, HD), (DH, D), (DH, D), (HD, D), (F, D), (F, D), (F, D)]
    scratch = [pltpu.VMEM(sh, BF) for sh in in_shapes] + [pltpu.VMEM(sh, BF) for sh in out_shapes] + [
        pltpu.SemaphoreType.DMA((9,)),
        pltpu.SemaphoreType.DMA((9,)),
        pltpu.VMEM((S, D), BF),
        pltpu.VMEM((HD, D), BF),
        pltpu.VMEM((32, D), BF),
        pltpu.VMEM((S, 16), BF),
        pltpu.VMEM((16, S), BF),
        pltpu.VMEM((S, 32), BF),
        pltpu.VMEM((32, S), BF),
        pltpu.VMEM((S // 2, RT), U32),
        pltpu.VMEM((S, RC), F32),
        pltpu.VMEM((S, RC), F32),
        pltpu.VMEM((2, 16, RT), BF),
        pltpu.VMEM((32, RT), BF),
        pltpu.VMEM((16, RT), BF),
        pltpu.VMEM((16, RT), BF),
        pltpu.VMEM((32, RT), F32),
        pltpu.VMEM((16, RT), F32),
        pltpu.VMEM((HD, TQ), BF),
        pltpu.VMEM((HD, S), BF),
        pltpu.VMEM((16, S), F32),
        pltpu.VMEM((16, S), F32),
        pltpu.VMEM((S, D), F32),
        pltpu.VMEM((HD, D), F32),
        pltpu.VMEM((F, D), F32),
        pltpu.VMEM((F, D), F32),
        pltpu.VMEM((F, D), F32),
    ] + [pltpu.VMEM((KBB // 2, RC), U32) for _ in range(NDS)]
    return kernel, scratch


def build(**overrides):
    cfg = dict(DEFAULT_CFG)
    cfg.update(overrides)
    kernel, scratch = _make_kernel(cfg)

    def fn(A_x, A_wq, A_wk, A_wv, A_wo, B_x, B_w1, B_w3, B_w2, grad_out):
        x = A_x.reshape(S, D)
        g = grad_out.reshape(S, D)
        out_shape = (
            jax.ShapeDtypeStruct((S, D), BF), jax.ShapeDtypeStruct((S, D), BF),
            jax.ShapeDtypeStruct((D, HD), BF), jax.ShapeDtypeStruct((DH, D), BF), jax.ShapeDtypeStruct((DH, D), BF),
            jax.ShapeDtypeStruct((HD, D), BF), jax.ShapeDtypeStruct((F, D), BF), jax.ShapeDtypeStruct((F, D), BF),
            jax.ShapeDtypeStruct((F, D), BF),
        )
        outs = pl.pallas_call(
            kernel, out_shape=out_shape, scratch_shapes=scratch,
            in_specs=[pl.BlockSpec(memory_space=pl.ANY)] * 9,
            out_specs=tuple(pl.BlockSpec(memory_space=pl.ANY) for _ in range(9)),
            compiler_params=pltpu.CompilerParams(vmem_limit_bytes=120 * 1024 * 1024),
        )(x, A_wq, A_wk.T, A_wv.T, A_wo, B_w1.T, B_w3.T, B_w2, g)
        h2, dx, dwq, dwkt, dwvt, dwo, dw1t, dw3t, dw2 = outs
        return (h2.reshape(1, S, D), dx.reshape(1, S, D), dwq, dwkt.T, dwvt.T, dwo, dw1t.T, dw3t.T, dw2)
    return fn


_impl = build()


@jax.jit
def pallas_sequential_preLN__grouped_kv_mqa__glu_gated_swiglu__prompt_kernel(
    A_x, A_wq, A_wk, A_wv, A_wo, B_x, B_w1, B_w3, B_w2, grad_out,
):
    return _impl(A_x, A_wq, A_wk, A_wv, A_wo, B_x, B_w1, B_w3, B_w2, grad_out)
```

```python
import contextlib
import jax
import jax.numpy as jnp
from jax import lax
from jax.experimental import pallas as pl
from jax.experimental.pallas import tpu as pltpu

F32 = jnp.float32
BF = jnp.bfloat16
U32 = jnp.uint32

S, D, H, DH, F = 2048, 512, 32, 16, 1376
HD = H * DH
EPS = 1e-5
SCALE = DH ** -0.5
NEG = -1e30

NT_DIMS = (((1,), (1,)), ((), ()))
TN_DIMS = (((0,), (0,)), ((), ()))
TT_DIMS = (((0,), (1,)), ((), ()))

DEFAULT_CFG = dict(
    TQ=256,
    RC=512,
    RCB=512,
    KBF=128,
    KBB=128,
    RB=16,
    RC1=256,
    BWD_ORDER='dv,dk,dq',
    FWD_ORDER='pc',
    BWD_DIST=2,
    BWD_APOS=0,
    PROFILE=False,
)


def _dg(a, b, dims):
    return lax.dot_general(a, b, dims, preferred_element_type=F32)


def _nn(a, b):
    return jnp.dot(a, b, preferred_element_type=F32)


def _ln_stats(x):
    mu = jnp.mean(x, axis=-1, keepdims=True)
    xc = x - mu
    var = jnp.mean(xc * xc, axis=-1, keepdims=True)
    rstd = lax.rsqrt(var + EPS)
    return xc * rstd, rstd


def _ln_bwd(dy, xhat, rstd):
    m1 = jnp.mean(dy, axis=-1, keepdims=True)
    m2 = jnp.mean(dy * xhat, axis=-1, keepdims=True)
    return rstd * (dy - m1 - xhat * m2)


def _make_kernel(cfg):
    TQ, RC, KBF, KBB, RB, RC1 = cfg['TQ'], cfg['RC'], cfg['KBF'], cfg['KBB'], cfg['RB'], cfg['RC1']
    NT = S // TQ
    RT = H * TQ
    NC = RT // RC
    RCB = cfg['RCB']
    NCB = RT // RCB
    NKBF = S // KBF
    NKBB = S // KBB
    BWD_ORDER = cfg['BWD_ORDER'].split(',')
    BWD_DIST = cfg['BWD_DIST']
    BWD_APOS = cfg['BWD_APOS']
    NDS = min(n for n in range(BWD_DIST + 1, NKBB + 1) if NKBB % n == 0)

    def scope(name):
        return jax.named_scope(name) if cfg['PROFILE'] else contextlib.nullcontext()

    def kernel(x_hbm, wq_hbm, wkt_hbm, wvt_hbm, wo_hbm, w1t_hbm, w3t_hbm, w2_hbm, g_hbm,
               h2_hbm, dx_hbm, dwq_hbm, dwkt_hbm, dwvt_hbm, dwo_hbm, dw1t_hbm, dw3t_hbm, dw2_hbm,
               x_ref, wq_ref, wkt_ref, wvt_ref, wo_ref, w1t_ref, w3t_ref, w2_ref, g_ref,
               h2_ref, dx_ref, dwq_ref, dwkt_ref, dwvt_ref, dwo_ref, dw1t_ref, dw3t_ref, dw2_ref,
               in_sems, out_sems,
               xn_scr, wqT_scr, wkvT_scr, k_scr, kT_scr, vaug_scr, vT_scr,
               p_scr, sA, sB,
               qcat_scr, doa_scr, qn_scr, don_scr, ol_scr, dqc_scr, oT_scr,
               dqT_scr, dkT_scr, dvT_scr, dh_scr,
               dwo_acc, dw1t_acc, dw3t_acc, dw2_acc, *dsb):
        in_pairs = [(x_hbm, x_ref), (wq_hbm, wq_ref), (wkt_hbm, wkt_ref), (wvt_hbm, wvt_ref), (wo_hbm, wo_ref),
                    (w1t_hbm, w1t_ref), (w3t_hbm, w3t_ref), (w2_hbm, w2_ref), (g_hbm, g_ref)]
        in_copies = [pltpu.make_async_copy(src, dst, in_sems.at[i]) for i, (src, dst) in enumerate(in_pairs)]
        for cp in in_copies:
            cp.start()

        with scope('prologue'):
            doa_scr[...] = jnp.zeros_like(doa_scr)
            dkT_scr[...] = jnp.zeros_like(dkT_scr)
            dvT_scr[...] = jnp.zeros_like(dvT_scr)
            dwo_acc[...] = jnp.zeros_like(dwo_acc)
            dw1t_acc[...] = jnp.zeros_like(dw1t_acc)
            dw3t_acc[...] = jnp.zeros_like(dw3t_acc)
            dw2_acc[...] = jnp.zeros_like(dw2_acc)
            row = lax.broadcasted_iota(jnp.int32, (16, S), 0)
            vT_scr[16:32, :] = jnp.where(row == 0, 1.0, 0.0).astype(BF)

            for cp in in_copies[1:4]:
                cp.wait()
            wqT_scr[...] = wq_ref[...].T
            wkvT_scr[0:16, :] = wkt_ref[...]
            wkvT_scr[16:32, :] = wvt_ref[...]

            in_copies[0].wait()

            def ln1_body(i, c):
                r = pl.ds(pl.multiple_of(i * RC1, RC1), RC1)
                xhat, _ = _ln_stats(x_ref[r, :].astype(F32))
                xn_scr[r, :] = xhat.astype(BF)
                return c
            lax.fori_loop(0, S // RC1, ln1_body, 0)

            xn_all = xn_scr[...]
            kv = _dg(xn_all, wkvT_scr[...], NT_DIMS)
            k_scr[...] = kv[:, 0:16].astype(BF)
            lane = lax.broadcasted_iota(jnp.int32, (S, 16), 1)
            ones2 = jnp.where(lane < 2, 1.0, 0.0).astype(F32)
            vaug_scr[...] = jnp.concatenate([kv[:, 16:32], ones2], axis=1).astype(BF)
            kvT = _dg(wkvT_scr[...], xn_all, NT_DIMS)
            kT_scr[...] = kvT[0:16, :].astype(BF)
            vT_scr[0:16, :] = kvT[16:32, :].astype(BF)

        def compute_qcat(t, slot):
            xn_t = xn_scr[pl.ds(pl.multiple_of(t * TQ, TQ), TQ), :]
            qT = _dg(wqT_scr[...], xn_t, NT_DIMS) * SCALE
            for h in range(H):
                qcat_scr[slot, :, h * TQ:(h + 1) * TQ] = qT[16 * h:16 * h + 16, :].astype(BF)

        def qt_chunk(slot, c):
            return qcat_scr[slot, :, pl.ds(pl.multiple_of(c * RC, 128), RC)]

        def produce(kb, qt, buf, macc):
            r0 = kb * KBF
            s_new = _nn(k_scr[pl.ds(r0, KBF), :], qt)
            buf[pl.ds(r0, KBF), :] = s_new
            return jnp.maximum(macc, jnp.max(s_new.reshape(KBF // RB, RB, RC), axis=0))

        def consume(kb, c_cur, buf, m, acc, lacc):
            r0 = kb * KBF
            p32 = jnp.exp(buf[pl.ds(r0, KBF), :] - m)
            lacc = lacc + jnp.sum(p32.reshape(KBF // RB, RB, RC), axis=0)
            p = p32.astype(BF)
            p_scr[pl.ds(kb * KBF // 2, KBF // 2),
                  pl.ds(pl.multiple_of(c_cur * RC, 128), RC)] = pltpu.bitcast(p, U32)
            return acc + _nn(vT_scr[0:16, pl.ds(r0, KBF)], p), lacc

        def first(qt, buf):
            macc = jnp.full((RB, RC), NEG, F32)
            for kb in range(NKBF):
                macc = produce(kb, qt, buf, macc)
            return jnp.max(macc, axis=0, keepdims=True)

        def piped(c_cur, bufC, mC, qt_nxt, bufN):
            macc = jnp.full((RB, RC), NEG, F32)
            acc = jnp.zeros((16, RC), F32)
            lacc = jnp.zeros((RB, RC), F32)
            for kb in range(NKBF):
                macc = produce(kb, qt_nxt, bufN, macc)
                acc, lacc = consume(kb, c_cur, bufC, mC, acc, lacc)
            cs = pl.ds(pl.multiple_of(c_cur * RC, 128), RC)
            ol_scr[0:16, cs] = acc
            ol_scr[16:24, cs] = jnp.broadcast_to(jnp.sum(lacc, axis=0, keepdims=True), (8, RC))
            return jnp.max(macc, axis=0, keepdims=True)

        compute_qcat(0, 0)
        m_init = first(qt_chunk(0, 0), sA)
        for cp in in_copies[4:]:
            cp.wait()

        def h2_copy(t):
            r = pl.ds(pl.multiple_of(t * TQ, TQ), TQ)
            return pltpu.make_async_copy(h2_ref.at[r, :], h2_hbm.at[r, :], out_sems.at[0])

        def tile_body(t, mA):
            rows = pl.ds(pl.multiple_of(t * TQ, TQ), TQ)
            cols = pl.ds(pl.multiple_of(t * TQ, TQ), TQ)
            slot = lax.rem(t, 2)
            nslot = 1 - slot

            with scope('qT'):
                compute_qcat(jnp.minimum(t + 1, NT - 1), nslot)

            with scope('attn_fwd'):
                def pair_body(c2, mA):
                    c = 2 * c2
                    mB = piped(c, sA, mA, qt_chunk(slot, c + 1), sB)
                    return piped(c + 1, sB, mB, qt_chunk(slot, c + 2), sA)
                mA = lax.fori_loop(0, NC // 2 - 1, pair_body, mA)
                mB = piped(NC - 2, sA, mA, qt_chunk(slot, NC - 1), sB)
                mA_next = piped(NC - 1, sB, mB, qt_chunk(nslot, 0), sA)

            with scope('norm'):
                ol = ol_scr[...]
                inv_l = 1.0 / ol[16:17, :]
                o_cat = ol[0:16, :] * inv_l
                for h in range(H):
                    oT_scr[16 * h:16 * h + 16, :] = o_cat[:, h * TQ:(h + 1) * TQ].astype(BF)
                oT = oT_scr[...]

            with scope('dense_fwd'):
                x_t = x_ref[rows, :].astype(F32)
                h1 = x_t + _dg(oT, wo_ref[...], TN_DIMS)
                hhat, rstd2 = _ln_stats(h1)
                hn = hhat.astype(BF)
                gate = _dg(hn, w1t_ref[...], NT_DIMS)
                up = _dg(hn, w3t_ref[...], NT_DIMS)
                sig = jax.nn.sigmoid(gate)
                silu = gate * sig
                a_bf = (silu * up).astype(BF)
                h2 = h1 + _nn(a_bf, w2_ref[...])
                h2_ref[rows, :] = h2.astype(BF)
                h2_copy(t).start()

            with scope('dense_bwd'):
                g_t = g_ref[rows, :]
                da = _dg(g_t, w2_ref[...], NT_DIMS)
                dw2_acc[...] += _dg(a_bf, g_t, TN_DIMS)
                dup = (da * silu).astype(BF)
                dgate = (da * up * (sig * (1.0 + gate * (1.0 - sig)))).astype(BF)
                dw1t_acc[...] += _dg(dgate, hn, TN_DIMS)
                dw3t_acc[...] += _dg(dup, hn, TN_DIMS)
                dhn = _nn(dgate, w1t_ref[...]) + _nn(dup, w3t_ref[...])
                dh = g_t.astype(F32) + _ln_bwd(dhn, hhat, rstd2)
                dh_scr[rows, :] = dh
                dh_bf = dh.astype(BF)
                dwo_acc[...] += _nn(oT, dh_bf)
                doT = _dg(wo_ref[...], dh_bf, NT_DIMS)

            with scope('scatter'):
                for h in range(H):
                    dqc_scr[:, h * TQ:(h + 1) * TQ] = doT[16 * h:16 * h + 16, :]
                do_cat = dqc_scr[...]
                delta = jnp.sum(do_cat * o_cat, axis=0, keepdims=True)
                d_hi = delta.astype(BF)
                d_lo = (delta - d_hi.astype(F32)).astype(BF)
                doa_scr[0:16, :] = do_cat.astype(BF)
                doa_scr[16:17, :] = -d_hi
                doa_scr[17:18, :] = -d_lo
                don_scr[...] = (do_cat * inv_l).astype(BF)
                qn_scr[...] = (qcat_scr[slot].astype(F32) * inv_l).astype(BF)

            with scope('attn_bwd'):
                def loadp(kb, loc):
                    return pltpu.bitcast(p_scr[pl.ds(kb * KBB // 2, KBB // 2), pl.ds(loc, RCB)], BF)

                def stageA(kb, loc):
                    r0 = kb * KBB
                    gm = _nn(vaug_scr[pl.ds(r0, KBB), :], doa_scr[:, pl.ds(loc, RCB)])
                    dsb[kb % NDS][...] = pltpu.bitcast((loadp(kb, loc).astype(F32) * gm).astype(BF), U32)

                def chunk_body(c, cc):
                    loc = pl.multiple_of(c * RCB, 128)
                    loc_nxt = pl.multiple_of(jnp.minimum(c + 1, NCB - 1) * RCB, 128)
                    qn = qn_scr[:, pl.ds(loc, RCB)]
                    don = don_scr[:, pl.ds(loc, RCB)]

                    def stageB(kb, dq_acc):
                        r0 = kb * KBB
                        for pos, what in enumerate(BWD_ORDER + ['end']):
                            if pos == BWD_APOS:
                                if kb + BWD_DIST < NKBB:
                                    stageA(kb + BWD_DIST, loc)
                                else:
                                    stageA(kb + BWD_DIST - NKBB, loc_nxt)
                            if what == 'end':
                                continue
                            if what == 'dq':
                                ds = pltpu.bitcast(dsb[kb % NDS][...], BF)
                                dq_acc = dq_acc + _nn(kT_scr[:, pl.ds(r0, KBB)], ds)
                            elif what == 'dk':
                                ds = pltpu.bitcast(dsb[kb % NDS][...], BF)
                                dkT_scr[:, pl.ds(r0, KBB)] += _dg(qn, ds, NT_DIMS)
                            else:
                                dvT_scr[:, pl.ds(r0, KBB)] += _dg(don, loadp(kb, loc), NT_DIMS)
                        return dq_acc

                    dq_acc = jnp.zeros((16, RCB), F32)
                    for kb in range(NKBB):
                        dq_acc = stageB(kb, dq_acc)
                    dqc_scr[:, pl.ds(loc, RCB)] = dq_acc
                    return cc
                for kb in range(BWD_DIST):
                    stageA(kb, 0)
                lax.fori_loop(0, NCB, chunk_body, 0)

            dq_cat = dqc_scr[...] * (inv_l * SCALE)
            for h in range(H):
                dqT_scr[16 * h:16 * h + 16, cols] = dq_cat[:, h * TQ:(h + 1) * TQ].astype(BF)
            return mA_next

        lax.fori_loop(0, NT, tile_body, m_init)

        with scope('epilogue'):
            dwo_ref[...] = dwo_acc[...].astype(BF)
            dw1t_ref[...] = dw1t_acc[...].astype(BF)
            dw3t_ref[...] = dw3t_acc[...].astype(BF)
            dw2_ref[...] = dw2_acc[...].astype(BF)
            w_copies = [pltpu.make_async_copy(dwo_ref, dwo_hbm, out_sems.at[2]),
                        pltpu.make_async_copy(dw1t_ref, dw1t_hbm, out_sems.at[3]),
                        pltpu.make_async_copy(dw3t_ref, dw3t_hbm, out_sems.at[4]),
                        pltpu.make_async_copy(dw2_ref, dw2_hbm, out_sems.at[5])]
            for cp in w_copies:
                cp.start()

            xn_all = xn_scr[...]
            dqT_all = dqT_scr[...]
            doa_scr[0:16, 0:S] = dkT_scr[...].astype(BF)
            doa_scr[16:32, 0:S] = dvT_scr[...].astype(BF)
            dkvT = doa_scr[:, 0:S]
            dwq_ref[...] = _nn(dqT_all, xn_all).T.astype(BF)
            dwkvt = _nn(dkvT, xn_all)
            dwkt_ref[...] = dwkvt[0:16, :].astype(BF)
            dwvt_ref[...] = dwkvt[16:32, :].astype(BF)
            w_copies += [pltpu.make_async_copy(dwq_ref, dwq_hbm, out_sems.at[6]),
                         pltpu.make_async_copy(dwkt_ref, dwkt_hbm, out_sems.at[7]),
                         pltpu.make_async_copy(dwvt_ref, dwvt_hbm, out_sems.at[8])]
            for cp in w_copies[4:]:
                cp.start()

            def dx_copy(i):
                r = pl.ds(pl.multiple_of(i * RC1, RC1), RC1)
                return pltpu.make_async_copy(dx_ref.at[r, :], dx_hbm.at[r, :], out_sems.at[1])

            def ep_body(i, c):
                off = pl.multiple_of(i * RC1, RC1)
                r = pl.ds(off, RC1)
                dxn = (_dg(dqT_scr[:, pl.ds(off, RC1)], wqT_scr[...], TN_DIMS) +
                       _dg(doa_scr[:, pl.ds(off, RC1)], wkvT_scr[...], TN_DIMS))
                xhat, rstd1 = _ln_stats(x_ref[r, :].astype(F32))
                dx = dh_scr[r, :] + _ln_bwd(dxn, xhat, rstd1)
                dx_ref[r, :] = dx.astype(BF)
                dx_copy(i).start()
                return c
            lax.fori_loop(0, S // RC1, ep_body, 0)

            def wait_h2(t, c):
                h2_copy(t).wait()
                return c
            lax.fori_loop(0, NT, wait_h2, 0)

            def wait_dx(i, c):
                dx_copy(i).wait()
                return c
            lax.fori_loop(0, S // RC1, wait_dx, 0)
            for cp in w_copies:
                cp.wait()

    in_shapes = [(S, D), (D, HD), (DH, D), (DH, D), (HD, D), (F, D), (F, D), (F, D), (S, D)]
    out_shapes = [(S, D), (S, D), (D, HD), (DH, D), (DH, D), (HD, D), (F, D), (F, D), (F, D)]
    scratch = [pltpu.VMEM(sh, BF) for sh in in_shapes] + [pltpu.VMEM(sh, BF) for sh in out_shapes] + [
        pltpu.SemaphoreType.DMA((9,)),
        pltpu.SemaphoreType.DMA((9,)),
        pltpu.VMEM((S, D), BF),
        pltpu.VMEM((HD, D), BF),
        pltpu.VMEM((32, D), BF),
        pltpu.VMEM((S, 16), BF),
        pltpu.VMEM((16, S), BF),
        pltpu.VMEM((S, 32), BF),
        pltpu.VMEM((32, S), BF),
        pltpu.VMEM((S // 2, RT), U32),
        pltpu.VMEM((S, RC), F32),
        pltpu.VMEM((S, RC), F32),
        pltpu.VMEM((2, 16, RT), BF),
        pltpu.VMEM((32, RT), BF),
        pltpu.VMEM((16, RT), BF),
        pltpu.VMEM((16, RT), BF),
        pltpu.VMEM((24, RT), F32),
        pltpu.VMEM((16, RT), F32),
        pltpu.VMEM((HD, TQ), BF),
        pltpu.VMEM((HD, S), BF),
        pltpu.VMEM((16, S), F32),
        pltpu.VMEM((16, S), F32),
        pltpu.VMEM((S, D), F32),
        pltpu.VMEM((HD, D), F32),
        pltpu.VMEM((F, D), F32),
        pltpu.VMEM((F, D), F32),
        pltpu.VMEM((F, D), F32),
    ] + [pltpu.VMEM((KBB // 2, RCB), U32) for _ in range(NDS)]
    return kernel, scratch


def build(**overrides):
    cfg = dict(DEFAULT_CFG)
    cfg.update(overrides)
    kernel, scratch = _make_kernel(cfg)

    def fn(A_x, A_wq, A_wk, A_wv, A_wo, B_x, B_w1, B_w3, B_w2, grad_out):
        x = A_x.reshape(S, D)
        g = grad_out.reshape(S, D)
        out_shape = (
            jax.ShapeDtypeStruct((S, D), BF), jax.ShapeDtypeStruct((S, D), BF),
            jax.ShapeDtypeStruct((D, HD), BF), jax.ShapeDtypeStruct((DH, D), BF), jax.ShapeDtypeStruct((DH, D), BF),
            jax.ShapeDtypeStruct((HD, D), BF), jax.ShapeDtypeStruct((F, D), BF), jax.ShapeDtypeStruct((F, D), BF),
            jax.ShapeDtypeStruct((F, D), BF),
        )
        outs = pl.pallas_call(
            kernel, out_shape=out_shape, scratch_shapes=scratch,
            in_specs=[pl.BlockSpec(memory_space=pl.ANY)] * 9,
            out_specs=tuple(pl.BlockSpec(memory_space=pl.ANY) for _ in range(9)),
            compiler_params=pltpu.CompilerParams(vmem_limit_bytes=120 * 1024 * 1024),
        )(x, A_wq, A_wk.T, A_wv.T, A_wo, B_w1.T, B_w3.T, B_w2, g)
        h2, dx, dwq, dwkt, dwvt, dwo, dw1t, dw3t, dw2 = outs
        return (h2.reshape(1, S, D), dx.reshape(1, S, D), dwq, dwkt.T, dwvt.T, dwo, dw1t.T, dw3t.T, dw2)
    return fn


_impl = build()


@jax.jit
def pallas_sequential_preLN__grouped_kv_mqa__glu_gated_swiglu__prompt_kernel(
    A_x, A_wq, A_wk, A_wv, A_wo, B_x, B_w1, B_w3, B_w2, grad_out,
):
    return _impl(A_x, A_wq, A_wk, A_wv, A_wo, B_x, B_w1, B_w3, B_w2, grad_out)
```
